```python
import os as _os
_os.environ.setdefault("JAX_PLATFORMS", "cpu")
import jax
import jax.numpy as jnp

def _softmax(x, axis=-1):
    return jax.nn.softmax(x, axis=axis)
def _gelu(x):
    return jax.nn.gelu(x, approximate=True)
def _silu(x):
    return jax.nn.silu(x)
def _sigmoid(x):
    return jax.nn.sigmoid(x)
def _layernorm(x, axis=-1, eps=1e-5):
    m = jnp.mean(x, axis=axis, keepdims=True)
    v = jnp.var(x, axis=axis, keepdims=True)
    return (x - m) / jnp.sqrt(v + eps)
def _scatter_add(tgt, idx, src, axis=0):
    return tgt.at[idx].add(src)
def _segment_sum(src, seg, n):
    return jax.ops.segment_sum(src, seg, n)
class _Rng:
    def __init__(self, key):
        self._k = key
    def _next(self):
        self._k, sub = jax.random.split(self._k)
        return sub
    def normal(self, shape):
        return jax.random.normal(self._next(), shape, dtype=jnp.bfloat16)
    def randint(self, lo, hi, shape):
        return jax.random.randint(self._next(), shape, lo, hi, dtype=jnp.int32)
    def uniform(self, shape, lo=0.0, hi=1.0):
        return jax.random.uniform(self._next(), shape, jnp.bfloat16, lo, hi)
    def permutation(self, n):
        return jax.random.permutation(self._next(), n)


kernel_name = 'sequential_preLN__softmax_full_mha__mixer_channel_mlp__prompt'

def setup_inputs():
    _rng = _Rng(jax.random.key(int.from_bytes(__import__("os").urandom(4), "little")))
    _w = (lambda a: (lambda t: t.astype(jnp.bfloat16) if jnp.issubdtype(t.dtype, jnp.floating) else t)(jnp.asarray(a)))
    def _A_setup():
        B, S, D = 1, 2048, 1024
        return {
            "x": _w((lambda *s: _rng.normal(s) * 0.05)(B, S, D)),
            "wqkv": _w((lambda *s: _rng.normal(s) * 0.05)(D, 3 * D)),
            "wo": _w((lambda *s: _rng.normal(s) * 0.05)(D, D)),
        }
    _A_in = _A_setup()

    def _B_setup():
        B, S, D, F = 1, 2048, 1024, 3584
        return {
            "x": _w((lambda *s: _rng.normal(s) * 0.05)(B, S, D)),
            "w1": _w((lambda *s: _rng.normal(s) * 0.8)(D, F) * (D ** -0.5)),
            "b1": _w((lambda *s: _rng.normal(s) * 0.8)(F)),
            "w2": _w((lambda *s: _rng.normal(s) * 0.8)(F, D) * (F ** -0.5)),
            "b2": _w((lambda *s: _rng.normal(s) * 0.05)(D)),
        }
    _B_in = _B_setup()

    return {
        "A_x": _A_in["x"],
        "A_wqkv": _A_in["wqkv"],
        "A_wo": _A_in["wo"],
        "B_x": _B_in["x"],
        "B_w1": _B_in["w1"],
        "B_b1": _B_in["b1"],
        "B_w2": _B_in["w2"],
        "B_b2": _B_in["b2"],
    }

def reference(A_x, A_wqkv, A_wo, B_x, B_w1, B_b1, B_w2, B_b2):
    def _A_ref(x, wqkv, wo):
        B, S, D = x.shape
        H = 32; Dh = D // H
        qkv = (lambda x, *d: x.transpose(*d))((x @ wqkv).reshape(B, S, 3, H, Dh), 2, 0, 3, 1, 4)
        q, k, v = qkv[0], qkv[1], qkv[2]
        scale = Dh ** -0.5
        scores = jnp.einsum("bhqd,bhkd->bhqk", q, k) * scale
        p = _softmax(scores, axis=-1)
        o = jnp.einsum("bhqk,bhkd->bhqd", p, v)
        return (lambda x, *d: x.transpose(*d))(o, 0, 2, 1, 3).reshape(B, S, D) @ wo

    def _B_ref(x, w1, b1, w2, b2):
        y = _layernorm(x, axis=-1)
        h = _gelu(jnp.einsum("bsd,df->bsf", y, w1) + b1)
        return jnp.einsum("bsf,fd->bsd", h, w2) + b2

    x = A_x
    h = x + _A_ref(_layernorm(x, axis=-1), A_wqkv, A_wo)
    h2 = h + _B_ref(_layernorm(h, axis=-1), B_w1, B_b1, B_w2, B_b2)
    return h2
```

```python
import functools
import math

import jax
import jax.numpy as jnp
from jax import lax
import jax.experimental.pallas as pl
import jax.experimental.pallas.tpu as pltpu

S, D, F, H, DH = 2048, 1024, 3584, 32, 32
G = D // 128
TM = 512
NB = S // TM
TC = 256
CK = 128
NC = S // CK
SKEW = 1
R = 32
FC = 512
EPS = 1e-5
QSCALE = (DH ** -0.5) * math.log2(math.e)
BF, F32 = jnp.bfloat16, jnp.float32
SCOPES = False


class _scope:
    def __init__(self, name):
        self.cm = jax.named_scope(name) if SCOPES else None

    def __enter__(self):
        if self.cm:
            self.cm.__enter__()

    def __exit__(self, *a):
        if self.cm:
            self.cm.__exit__(*a)


def _layernorm(x):
    m = jnp.mean(x, axis=-1, keepdims=True)
    xc = x - m
    v = jnp.mean(xc * xc, axis=-1, keepdims=True)
    return xc * lax.rsqrt(v + EPS)


def _gelu(x):
    c = math.sqrt(2.0 / math.pi)
    inner = x * (c + (c * 0.044715) * (x * x))
    hx = 0.5 * x
    return hx + hx * jnp.tanh(inner)


def _rows(i, n):
    return pl.ds(pl.multiple_of(i * n, n), n)


def _kernel(x_hbm, wqkv_hbm, wo_hbm, w1_hbm, b1_hbm, w2_hbm, b2_hbm, out_hbm,
            x_v, wqkv_v, wo_v, w1_v, b1_v, w2_v, b2_v,
            y_v, qvt_v, k_v, sa_v, sb_v, ot_v, l_v, o_v, h_v, out_v,
            sem_x, sem_w, sem_m, sem_o):
    x_cp = [pltpu.make_async_copy(x_hbm.at[pl.ds(r * TM, TM), :], x_v.at[pl.ds(r * TM, TM), :], sem_x.at[r])
            for r in range(NB)]
    w_cp = [pltpu.make_async_copy(wqkv_hbm.at[:, pl.ds(c * D, D)], wqkv_v.at[c], sem_w.at[c]) for c in range(3)]
    m_cp = [pltpu.make_async_copy(s, d, sem_m.at[i]) for i, (s, d) in enumerate(
        [(wo_hbm, wo_v), (w1_hbm, w1_v), (w2_hbm, w2_v), (b1_hbm, b1_v), (b2_hbm, b2_v)])]

    with _scope("A0"):
        x_cp[0].start()
        w_cp[1].start()
        x_cp[1].start()
        x_cp[0].wait()
        y_v[0:TM, :] = _layernorm(x_v[0:TM, :].astype(F32)).astype(BF)
        w_cp[1].wait()
        x_cp[2].start()
        x_cp[3].start()
        w_cp[0].start()
        w_cp[2].start()

    def x_wait(r):
        pltpu.make_async_copy(x_hbm.at[_rows(r, TM), :], x_v.at[_rows(r, TM), :], sem_x.at[r]).wait()

    def k_body(r, carry):
        rn = jnp.minimum(r + 1, NB - 1)

        @pl.when(r + 1 < NB)
        def _():
            x_wait(rn)

        a = jnp.dot(y_v[_rows(r, TM), :], wqkv_v[1], preferred_element_type=F32)
        for g in range(G):
            k_v[g, _rows(r, TM), :] = a[:, g * 128:(g + 1) * 128].astype(BF)
        y_next = _layernorm(x_v[_rows(rn, TM), :].astype(F32)).astype(BF)
        y_v[_rows(rn, TM), :] = y_next
        return carry
    with _scope("A1"):
        lax.fori_loop(0, NB, k_body, 0)

    w_cp[0].wait()
    w_cp[2].wait()
    for cp in m_cp:
        cp.start()

    def qv_body(i, carry):
        which, r = i // NB, i % NB
        scale = jnp.where(which == 0, QSCALE, 1.0).astype(F32)
        a = jnp.dot(y_v[_rows(r, TM), :], wqkv_v[2 * which], preferred_element_type=F32)
        for g in range(G):
            qvt_v[which, r, g] = (a[:, g * 128:(g + 1) * 128] * scale).T.astype(BF)
        return carry
    with _scope("A2"):
        lax.fori_loop(0, 2 * NB, qv_body, 0)

    bufs = (sa_v, sb_v)

    def q_weights(t, j):
        qb, g = t // G, t % G
        q = qvt_v[0, qb, g, 32 * j:32 * (j + 1), :]
        parts = []
        if j > 0:
            parts.append(jnp.zeros((32 * j, TM), BF))
        parts.append(q)
        if j < 3:
            parts.append(jnp.zeros((32 * (3 - j), TM), BF))
        return jnp.concatenate(parts, axis=0)

    def score_chunk(t, qw, c, dst, mp):
        s = jnp.dot(k_v[t % G, c * CK:(c + 1) * CK, :], qw, preferred_element_type=F32)
        dst[c * CK:(c + 1) * CK, :] = s
        for i in range(CK // 8):
            b = s[8 * i:8 * i + 8]
            mp = b if mp is None else jnp.maximum(mp, b)
        return mp

    with _scope("B0"):
        qw = q_weights(0, 0)
        mp = None
        for c in range(NC):
            mp = score_chunk(0, qw, c, bufs[0], mp)
        m0 = jnp.max(mp, axis=0, keepdims=True)
        qw = q_weights(0, 1)
        mp = None
        for c in range(SKEW):
            mp = score_chunk(0, qw, c, bufs[1], mp)
        ot_v[...] = jnp.zeros_like(ot_v)
        l_v[...] = jnp.ones_like(l_v)

    def finalize(t):
        qb, g = t // G, t % G
        inv = 1.0 / jnp.sum(l_v[...], axis=0, keepdims=True)
        ot = jnp.concatenate([ot_v[0:96, :], ot_v[96:128, :] * inv], axis=0)
        o_v[g, _rows(qb, TM), :] = ot.T.astype(BF)

    def b_body(t, carry):
        m_cur, mp = carry
        tn = jnp.minimum(t + 1, NB * G - 1)
        g = t % G
        sub = lax.broadcasted_iota(jnp.int32, (8, TM), 0)
        always = sub >= jnp.minimum(t, 0)
        always2 = sub < 8 + jnp.maximum(t, 0)
        qw = q_weights(t, 1)
        m_next = None
        lh, ah = [], []
        for j in range(4):
            l = None
            acc = None
            mb = jnp.broadcast_to(m_cur, (8, TM))
            for c in range(NC):
                u = j * NC + c
                hs, cs = divmod(u + NC + SKEW, NC)
                ts, js = (t, hs) if hs < 4 else (tn, hs - 4)
                if cs == 0:
                    qw = q_weights(ts, js)
                    mp = None
                mp = score_chunk(ts, qw, cs, bufs[hs % 2], mp)
                if cs == NC - 1:
                    m_next = jnp.max(mp, axis=0, keepdims=True)
                ps = []
                for k in range(CK // R):
                    mk = mb
                    if len(lh) >= 2:
                        mk = jnp.where(always, mk, lh[-2])
                    if k == 0 and u >= 2:
                        mk = jnp.where(always2, mk, ah[u - 2][0:8, :])
                    s = bufs[j % 2][c * CK + k * R:c * CK + (k + 1) * R, :]
                    p = jnp.exp2(s.reshape(R // 8, 8, TM) - mk[None])
                    for i in range(R // 8):
                        l = p[i] if l is None else l + p[i]
                    lh.append(l)
                    ps.append(p.reshape(R, TM).astype(BF))
                kb, ko = divmod(c * CK, TM)
                o = jnp.dot(qvt_v[1, kb, g, 32 * j:32 * (j + 1), ko:ko + CK], jnp.concatenate(ps, axis=0),
                            preferred_element_type=F32)
                ah.append(o)
                acc = o if acc is None else acc + o
                if u == 1:
                    finalize(jnp.maximum(t - 1, 0))
            if j < 3:
                ot_v[32 * j:32 * (j + 1), :] = acc * (1.0 / jnp.sum(l, axis=0, keepdims=True))
            else:
                ot_v[96:128, :] = acc
                l_v[...] = l
            m_cur = m_next
        return m_cur, mp
    with _scope("B"):
        lax.fori_loop(0, NB * G, b_body, (m0, mp))
        finalize(NB * G - 1)

    for cp in m_cp:
        cp.wait()

    def wo_body(r, carry):
        rows = _rows(r, TM)
        o = jnp.concatenate([o_v[g, rows, :] for g in range(G)], axis=1)
        h_v[rows, :] = x_v[rows, :].astype(F32) + jnp.dot(o, wo_v[...], preferred_element_type=F32)
        return carry
    with _scope("C1"):
        lax.fori_loop(0, NB, wo_body, 0)

    def out_copy(i):
        return pltpu.make_async_copy(out_v.at[_rows(i, TC), :], out_hbm.at[_rows(i, TC), :], sem_o.at[i])

    def mlp_body(i, carry):
        nxt = jnp.minimum(i + 1, S // TC - 1)
        y = y_v[_rows(i, TC), :]
        acc = h_v[_rows(i, TC), :] + b2_v[...].astype(F32)
        for c in range(F // FC):
            a = jnp.dot(y, w1_v[:, c * FC:(c + 1) * FC], preferred_element_type=F32)
            a = a + b1_v[:, c * FC:(c + 1) * FC].astype(F32)
            acc = acc + jnp.dot(_gelu(a).astype(BF), w2_v[c * FC:(c + 1) * FC, :], preferred_element_type=F32)
        out_v[_rows(i, TC), :] = acc.astype(BF)
        y_v[_rows(nxt, TC), :] = _layernorm(h_v[_rows(nxt, TC), :]).astype(BF)
        out_copy(i).start()
        return carry
    with _scope("C2"):
        y_v[0:TC, :] = _layernorm(h_v[0:TC, :]).astype(BF)
        lax.fori_loop(0, S // TC, mlp_body, 0)
    with _scope("outwait"):
        for i in range(S // TC):
            out_copy(i).wait()


@jax.jit
def pallas_sequential_preLN__softmax_full_mha__mixer_channel_mlp__prompt_kernel(A_x, A_wqkv, A_wo, B_x, B_w1, B_b1, B_w2, B_b2):
    del B_x
    any_spec = pl.BlockSpec(memory_space=pl.ANY)
    out = pl.pallas_call(
        _kernel,
        out_shape=jax.ShapeDtypeStruct((S, D), BF),
        in_specs=[any_spec] * 7,
        out_specs=any_spec,
        scratch_shapes=[
            pltpu.VMEM((S, D), BF),
            pltpu.VMEM((3, D, D), BF),
            pltpu.VMEM((D, D), BF),
            pltpu.VMEM((D, F), BF),
            pltpu.VMEM((1, F), BF),
            pltpu.VMEM((F, D), BF),
            pltpu.VMEM((1, D), BF),
            pltpu.VMEM((S, D), BF),
            pltpu.VMEM((2, NB, G, 128, TM), BF),
            pltpu.VMEM((G, S, 128), BF),
            pltpu.VMEM((S, TM), F32),
            pltpu.VMEM((S, TM), F32),
            pltpu.VMEM((128, TM), F32),
            pltpu.VMEM((8, TM), F32),
            pltpu.VMEM((G, S, 128), BF),
            pltpu.VMEM((S, D), F32),
            pltpu.VMEM((S, D), BF),
            pltpu.SemaphoreType.DMA((NB,)),
            pltpu.SemaphoreType.DMA((3,)),
            pltpu.SemaphoreType.DMA((5,)),
            pltpu.SemaphoreType.DMA((S // TC,)),
        ],
        compiler_params=pltpu.CompilerParams(vmem_limit_bytes=100 * 1024 * 1024),
        name="fused_block",
    )(A_x.reshape(S, D), A_wqkv, A_wo, B_w1, B_b1.reshape(1, F), B_w2, B_b2.reshape(1, D))
    return out.reshape(1, S, D)
```

```python
import functools
import math

import jax
import jax.numpy as jnp
from jax import lax
import jax.experimental.pallas as pl
import jax.experimental.pallas.tpu as pltpu

S, D, F, H, DH = 2048, 1024, 3584, 32, 32
G = D // 128
TM = 512
NB = S // TM
TC = 256
CK = 128
NC = S // CK
D2, F2 = D // 2, F // 2
FCH = ((0, 512), (512, 1024), (1024, 1536), (1536, 1792))
EPS = 1e-5
QSCALE = (DH ** -0.5) * math.log2(math.e)
BF, F32, I32 = jnp.bfloat16, jnp.float32, jnp.int32
SCOPES = False
CFG = dict(a1_lag=0, a1_start=10, a2_lag=0, c1_lag=4, c2_lag=0, c2_start=30, c2_stride=4, c2_skew=1,
           R=64, llag=2, alag=2, skew=1, fin=19, finu=16, a1_reload=1, tr_rows=32, a2_first=3, qre=16, xtie=0, split=1, pair=8, ahead=2)


class _scope:
    def __init__(self, name):
        self.cm = jax.named_scope(name) if SCOPES else None

    def __enter__(self):
        if self.cm:
            self.cm.__enter__()

    def __exit__(self, *a):
        if self.cm:
            self.cm.__exit__(*a)


def _ln_stats(x, stat_ref, r0=0):
    m = jnp.mean(x, axis=-1, keepdims=True)
    xc = x - m
    v = jnp.mean(xc * xc, axis=-1, keepdims=True)
    n = x.shape[0]
    rs = jnp.broadcast_to(lax.rsqrt(v + EPS), (n, 128))
    stat_ref[0, r0:r0 + n, :] = jnp.broadcast_to(m, (n, 128))
    stat_ref[1, r0:r0 + n, :] = rs
    return rs


def _ln_apply(quad, stat_ref, n):
    out = []
    for i in range(2):
        m = jnp.tile(stat_ref[0, i * (n // 2):(i + 1) * (n // 2), :], (1, D2 // 128))
        rs = jnp.tile(stat_ref[1, i * (n // 2):(i + 1) * (n // 2), :], (1, D2 // 128))
        out += [(quad(i, j) - m) * rs for j in range(2)]
    return out


def _gelu(x):
    c = math.sqrt(2.0 / math.pi)
    inner = x * (c + (c * 0.044715) * (x * x))
    hx = 0.5 * x
    return hx + hx * jnp.tanh(inner)


def _rows(i, n):
    return pl.ds(pl.multiple_of(i * n, n), n)


def _dot(a, b):
    return jnp.dot(a, b, preferred_element_type=F32)


def _pack(x):
    return pltpu.bitcast(x, jnp.int32)


def _unpack(x):
    return pltpu.bitcast(x, BF)


def _lhs_terms(a11, a12, a21, a22):
    return [t.astype(BF) for t in (a11 + a22, a21 + a22, a11, a22, a11 + a12, a21 - a11, a12 - a22)]


class _Order:
    def __init__(self, step):
        self.true = lax.broadcasted_iota(jnp.int32, (8, 128), 0) >= jnp.minimum(step, 0)

    def tie(self, x, dep):
        packed = x.dtype != F32
        v = pltpu.bitcast(x, F32) if packed else x
        reps = (v.shape[0] // 8, v.shape[1] // 128)
        v = jnp.where(jnp.tile(self.true, reps), v, jnp.tile(dep, reps))
        return pltpu.bitcast(v, x.dtype) if packed else v

    def tie_first(self, x, dep):
        r = 32 // x.dtype.itemsize
        first = self.tie(x[:r, :128], dep)
        if x.shape[1] > 128:
            first = jnp.concatenate([first, x[:r, 128:]], axis=1)
        return jnp.concatenate([first, x[r:]], axis=0)

    def join(self, dep, x):
        v = pltpu.bitcast(x, F32) if x.dtype != F32 else x
        for i in range(v.shape[0] // 8):
            for j in range(v.shape[1] // 128):
                t = v[8 * i:8 * i + 8, 128 * j:128 * j + 128]
                dep = t if dep is None else jnp.where(self.true, dep, t)
        return dep


class _Steps:
    def __init__(self, order, side, lag):
        self.order, self.side, self.lag, self.done = order, side, lag, []

    def __call__(self, a, b):
        if self.lag and len(self.done) >= self.lag and self.done[-self.lag]:
            dep = None
            for t in self.done[-self.lag]:
                dep = self.order.join(dep, t)
            a = self.order.tie_first(a, dep)
        d = _dot(a, b)
        job = self.side.get(len(self.done))
        self.done.append(job(d[0:8, 0:128]) if job else None)
        return d


def _rhs_terms(w_ref, t_ref, i, n, cols=None, order=None, dep=None):
    k2, n2 = w_ref.shape[0] // 2, w_ref.shape[1] // 2
    c0, c1 = cols or (0, n2)
    top, bot = _rows(i, n), pl.ds(pl.multiple_of(k2 + i * n, n), n)
    load = lambda v: (v if dep is None else order.tie(v, dep)).astype(F32)
    b11, b12 = load(w_ref[top, c0:c1]), load(w_ref[top, n2 + c0:n2 + c1])
    b21, b22 = load(w_ref[bot, c0:c1]), load(w_ref[bot, n2 + c0:n2 + c1])
    terms = [t.astype(BF) for t in (b11 + b22, b12 - b22, b21 - b11, b11 + b12, b21 + b22)]
    for s, t in enumerate(terms):
        t_ref[s, _rows(i, n // 2), c0:c1] = _pack(t)
    return terms


def _rhs(w_ref, t_ref, i, rows, cols):
    k2, n2 = w_ref.shape[0] // 2, w_ref.shape[1] // 2
    (r0, r1), (c0, c1) = rows, cols
    if i == 1:
        return w_ref[r0:r1, c0:c1]
    if i == 4:
        return w_ref[k2 + r0:k2 + r1, n2 + c0:n2 + c1]
    return _unpack(t_ref[{0: 0, 2: 1, 3: 2, 5: 3, 6: 4}[i], r0 // 2:r1 // 2, c0:c1])


def _strassen(prod, emit):
    m3, m5 = prod(2), prod(4)
    emit(0, 1, m3 + m5)
    m2, m4 = prod(1), prod(3)
    emit(1, 0, m2 + m4)
    t22, t11 = m3 - m2, m4 - m5
    m1, m7 = prod(0), prod(6)
    emit(0, 0, t11 + m1 + m7)
    emit(1, 1, t22 + m1 + prod(5))


def _strassen_tiles(step, lhs, w_ref, t_ref, cols, emit):
    for c in range(cols[0], cols[1], 128):
        _strassen(lambda i: step(lhs(i), _rhs(w_ref, t_ref, i, (0, D2), (c, c + 128))),
                  functools.partial(emit, c // 128))


def _kernel(x_hbm, wqkv_hbm, wo_hbm, w1_hbm, b1_hbm, w2_hbm, b2_hbm, out_hbm,
            x_v, w_v, wt_v, w1_v, w1t_v, b1_v, w2_v, w2t_v, b2_v,
            y_v, qvt_v, k_v, sa_v, sb_v, ot_v, l_v, o_v, stat_v, out_v,
            sem_x, sem_w, sem_k, sem_m, sem_o):
    x_cp = [pltpu.make_async_copy(x_hbm.at[pl.ds(r * TM, TM), :], x_v.at[pl.ds(r * TM, TM), :], sem_x.at[r])
            for r in range(NB)]
    w_cp = {c: pltpu.make_async_copy(wqkv_hbm.at[:, pl.ds(c * D, D)], w_v.at[c], sem_w.at[c]) for c in (0, 2)}
    w_cp[3] = pltpu.make_async_copy(wo_hbm, w_v.at[3], sem_w.at[3])
    m_cp = [pltpu.make_async_copy(s, d, sem_m.at[i]) for i, (s, d) in enumerate(
        [(w1_hbm, w1_v), (w2_hbm, w2_v), (b1_hbm, b1_v), (b2_hbm, b2_v.at[pl.ds(0, D)])])]
    full = (0, D2)
    AHEAD = CFG["ahead"]

    def half_rows(r, n, i):
        return pl.ds(pl.multiple_of(r * n + i * (n // 2), n // 2), n // 2)

    def wk_copy(i, half):
        rows = pl.ds(pl.multiple_of(half * D2 + i * 128, 128), 128)
        return pltpu.make_async_copy(wqkv_hbm.at[rows, pl.ds(D, D)], w_v.at[1, rows, :], sem_k.at[2 * i + half])

    def wk_start(i):
        wk_copy(i, 0).start()
        wk_copy(i, 1).start()

    def wk_wait(i):
        wk_copy(i, 0).wait()
        wk_copy(i, 1).wait()
        pl.when(i + AHEAD < D2 // 128)(lambda: wk_start(i + AHEAD))
        pl.when(i + AHEAD == D2 // 128)(x_cp[1].start)

    def transform(c, wait=None):
        n = CFG["tr_rows"]

        def body(i, carry):
            if wait:
                pl.when(i % (128 // n) == 0)(lambda: wait(i // (128 // n)))
            _rhs_terms(w_v.at[c], wt_v.at[c], i, n, None, _Order(i), jnp.zeros((8, 128), F32))
            return carry
        lax.fori_loop(0, D2 // n, body, 0)

    def score_store(p, rows, s):
        if CFG["split"]:
            sa_v[rows, 256 * p:256 * (p + 1)] = s[:, :256]
            sb_v[rows, 256 * p:256 * (p + 1)] = s[:, 256:]
        else:
            (sa_v, sb_v)[p][rows, :] = s

    def score_load(p, rows):
        if CFG["split"]:
            return jnp.concatenate([sa_v[rows, 256 * p:256 * (p + 1)], sb_v[rows, 256 * p:256 * (p + 1)]], axis=1)
        return (sa_v, sb_v)[p][rows, :]

    with _scope("A0"):
        x_cp[0].start()
        for i in range(AHEAD - 1):
            wk_start(i)
        score_store(1, slice(0, S), jnp.zeros((S, TM), F32))
        ot_v[...] = jnp.zeros_like(ot_v)
        l_v[...] = jnp.ones_like(l_v)
        x_cp[0].wait()
        wk_start(AHEAD - 1)
        _ln_stats(x_v[0:TM, :].astype(F32), stat_v)
        transform(1, wk_wait)
        x_cp[2].start()
        x_cp[3].start()
        w_cp[0].start()
        w_cp[2].start()

    def x_wait(r):
        pltpu.make_async_copy(x_hbm.at[_rows(r, TM), :], x_v.at[_rows(r, TM), :], sem_x.at[r]).wait()

    def k_body(r, carry):
        rn = jnp.minimum(r + 1, NB - 1)

        @pl.when(r + 1 < NB)
        def _():
            x_wait(rn)

        @pl.when(r == 1)
        def _():
            w_cp[3].start()
            m_cp[0].start()

        def emit(n, i, j, c):
            k_v[4 * j + n, half_rows(r, TM // 2, i), :] = _pack(c.astype(BF))
        order = _Order(r)
        whole = (lambda v: order.tie(v, jnp.zeros((8, 128), F32))) if CFG["xtie"] else (lambda v: v)
        lhs = _lhs_terms(*_ln_apply(
            lambda i, j: whole(x_v[half_rows(r, TM, i), j * D2:(j + 1) * D2]).astype(F32), stat_v, TM))
        for i in range(7):
            y_v[r, i] = _pack(lhs[i])

        def stats(k, dep):
            x = order.tie(x_v[_rows(16 * rn + k, 32), :], dep).astype(F32)
            return [_ln_stats(x, stat_v, k * 32)]
        side = {CFG["a1_start"] + k: functools.partial(stats, k) for k in range(16)}
        _strassen_tiles(_Steps(order, side, CFG["a1_lag"]), lambda i: _unpack(y_v[r, i]) if CFG["a1_reload"] else lhs[i],
                        w_v.at[1], wt_v.at[1], full, emit)
        return carry
    with _scope("A1"):
        lax.fori_loop(0, NB, k_body, 0)

    with _scope("A1t"):
        w_cp[0].wait()
        transform(0)
        w_cp[2].wait()
        w_cp[3].wait()
        m_cp[0].wait()
        for cp in m_cp[1:]:
            cp.start()

    def qv_body(it, carry):
        which, r = it // NB, it % NB
        scale = jnp.where(which == 0, QSCALE, 1.0).astype(F32)

        def emit(n, i, j, c):
            qvt_v[which, r, 4 * j + n, :, i * (TM // 2):(i + 1) * (TM // 2)] = _pack((c * scale).T.astype(BF))
        order = _Order(it)
        side = [functools.partial(_rhs_terms, w_v.at[2 + which], wt_v.at[2 + which], 8 * r + i, 16, None, order)
                for i in range(8)]
        side += [functools.partial(_rhs_terms, w1_v, w1t_v, 4 * it + i, 16, c, order)
                 for i in range(4) for c in FCH]
        _strassen_tiles(_Steps(order, dict(enumerate(side, CFG["a2_first"])), CFG["a2_lag"]), lambda i: _unpack(y_v[r, i]),
                        w_v.at[2 * which], wt_v.at[2 * which], full, emit)
        return carry
    with _scope("A2"):
        lax.fori_loop(0, 2 * NB, qv_body, 0)

    bufs = (sa_v, sb_v)
    SKEW, R = CFG["skew"], CFG["R"]

    def q_weights(t, j):
        qb, g = t // G, t % G
        q = _unpack(qvt_v[0, qb, g, 16 * j:16 * (j + 1), :])
        parts = []
        if j > 0:
            parts.append(jnp.zeros((32 * j, TM), BF))
        parts.append(q)
        if j < 3:
            parts.append(jnp.zeros((32 * (3 - j), TM), BF))
        return jnp.concatenate(parts, axis=0)

    def score_chunk(t, qw, c, dst, mp):
        s = _dot(_unpack(k_v[t % G, c * CK // 2:(c + 1) * CK // 2, :]), qw)
        score_store(dst, slice(c * CK, (c + 1) * CK), s)
        for i in range(CK // 8):
            b = s[8 * i:8 * i + 8]
            mp = b if mp is None else jnp.maximum(mp, b)
        return mp

    def softmax_chunk(tt, j, c, mb, l, link=None):
        ps = []
        for k in range(CK // R):
            s = score_load(j % 2, slice(c * CK + k * R, c * CK + (k + 1) * R))
            p = jnp.exp2(s.reshape(R // 8, 8, TM) - (link(k, mb, l) if link else mb)[None])
            if CFG["pair"]:
                n = CFG["pair"]
                for i in range(0, R // 8, n):
                    t = [p[i + e] for e in range(n)]
                    while len(t) > 1:
                        t = [a + b for a, b in zip(t[0::2], t[1::2])]
                    l = t[0] if l is None else l + t[0]
            else:
                for i in range(R // 8):
                    l = p[i] if l is None else l + p[i]
            ps.append(p.reshape(R, TM))
        kb, ko = divmod(c * CK, TM)
        vt = _unpack(qvt_v[1, kb, tt % G, 16 * j:16 * (j + 1), ko:ko + CK])
        return _dot(vt, jnp.concatenate(ps, axis=0).astype(BF)), l

    def normalise(acc, l):
        return acc * (1.0 / jnp.sum(l, axis=0, keepdims=True))

    def finalize(t, acc, l):
        ot = jnp.concatenate([ot_v[0:64, :], normalise(ot_v[64:96, :], l_v[...]), normalise(acc, l)], axis=0)
        o = ot.T
        o_v[t % G, _rows(t // G, TM), :] = o
        return jnp.concatenate([o[i + 120:i + 128, :] for i in range(0, TM, 128)], axis=1)

    def b_body(t, carry):
        m_cur, mp = carry
        tp, tn = jnp.maximum(t - 1, 0), jnp.minimum(t + 1, NB * G - 1)
        sub = lax.broadcasted_iota(jnp.int32, (8, TM), 0)
        always = sub >= jnp.minimum(t, 0)
        always2 = sub < 8 + jnp.maximum(t, 0)
        qw = q_weights(t, 0)
        m_next = finalized = None
        lh, ah = [], []
        for step, (tc, j) in enumerate(((tp, 3), (t, 0), (t, 1), (t, 2))):
            l = acc = None
            mb = jnp.broadcast_to(m_cur, (8, TM))
            for c in range(NC):
                u = step * NC + c
                hs, cs = divmod(u + SKEW, NC)
                ts, js = (t, hs) if hs < 4 else (tn, hs - 4)
                if cs == 0:
                    mp = None
                if cs % CFG["qre"] == 0:
                    qw = q_weights(ts, js)
                mp = score_chunk(ts, qw, cs, hs % 2, mp)
                if cs == NC - 1:
                    m_next = jnp.max(mp, axis=0, keepdims=True)

                def link(k, mk, l):
                    if l is not None:
                        lh.append(l)
                    if len(lh) >= CFG["llag"]:
                        mk = jnp.where(always, mk, lh[-CFG["llag"]])
                    if k == 0 and u >= CFG["alag"]:
                        mk = jnp.where(always2, mk, ah[u - CFG["alag"]][0:8, :])
                    if k == 1 and u == CFG["fin"]:
                        mk = jnp.where(always2, mk, finalized)
                    return mk
                o, l = softmax_chunk(tc, j, c, mb, l, link)
                ah.append(o)
                acc = o if acc is None else acc + o
            lh.append(l)
            if j == 3:
                finalized = finalize(tc, acc, l)
            elif j < 2:
                ot_v[32 * j:32 * (j + 1), :] = normalise(acc, l)
            else:
                ot_v[64:96, :] = acc
                l_v[...] = l
            m_cur = m_next
        return m_cur, mp

    with _scope("B"):
        qw = q_weights(0, 0)
        mp = None
        for c in range(SKEW):
            mp = score_chunk(0, qw, c, 0, mp)
        m_last, _ = lax.fori_loop(0, NB * G, b_body, (jnp.zeros((1, TM), F32), mp))
    with _scope("B1"):
        l = acc = None
        for c in range(NC):
            o, l = softmax_chunk(NB * G - 1, 3, c, jnp.broadcast_to(m_last, (8, TM)), l)
            acc = o if acc is None else acc + o
        finalize(NB * G - 1, acc, l)

    h_v = bufs
    for cp in m_cp[1:]:
        cp.wait()

    def wo_body(r, carry):
        quad = [jnp.concatenate([o_v[4 * j + g, half_rows(r, TM, i), :] for g in range(G // 2)], axis=1)
                for i in range(2) for j in range(2)]
        lhs = _lhs_terms(*quad)

        def emit(n, i, j, c):
            rows = half_rows(r, TM, i)
            h_v[j][rows, n * 128:(n + 1) * 128] = x_v[rows, j * D2 + n * 128:j * D2 + (n + 1) * 128].astype(F32) + c
        order = _Order(r)
        side = {i: functools.partial(_rhs_terms, w2_v, w2t_v, 28 * r + i, 16, None, order) for i in range(28)}
        _strassen_tiles(_Steps(order, side, CFG["c1_lag"]), lambda i: lhs[i], w_v.at[3], wt_v.at[3], full, emit)
        return carry
    with _scope("C1"):
        lax.fori_loop(0, NB, wo_body, 0)

    def out_copy(i):
        return pltpu.make_async_copy(out_v.at[_rows(i, TC), :], out_hbm.at[_rows(i, TC), :], sem_o.at[i])

    def mlp_body(it, carry):
        b1 = b1_v[...].astype(F32).reshape(1, F)
        b2 = b2_v[pl.ds(0, D)].astype(F32).reshape(1, D)
        y2 = _lhs_terms(*_ln_apply(lambda i, j: h_v[j][half_rows(it, TC, i), :], stat_v, TC))
        order = _Order(it)

        def stats_next(k, dep):
            rows = _rows(8 * jnp.minimum(it + 1, S // TC - 1) + k, 32)
            h = order.tie(jnp.concatenate([h_v[0][rows, :], h_v[1][rows, :]], axis=1), dep)
            return [_ln_stats(h, stat_v, 32 * k)]
        step = _Steps(order, {CFG["c2_start"] + CFG["c2_stride"] * k: functools.partial(stats_next, k)
                              for k in range(8)}, CFG["c2_lag"])

        def hidden(cols):
            gq = {}

            def emit(n, i, j, c):
                gq[n, i, j] = _gelu(c + b1[:, j * F2 + n * 128:j * F2 + (n + 1) * 128])
            _strassen_tiles(step, lambda i: y2[i], w1_v, w1t_v, cols, emit)
            tiles = [_lhs_terms(gq[n, 0, 0], gq[n, 0, 1], gq[n, 1, 0], gq[n, 1, 1])
                     for n in range(cols[0] // 128, cols[1] // 128)]
            return [jnp.concatenate([t[i] for t in tiles], axis=1) for i in range(7)]

        acc = {}

        def project(cols, g, last):
            width = 128 * 512 // (cols[1] - cols[0])
            for c in range(0, D2, width):
                def prod(i):
                    n = step(g[i], _rhs(w2_v, w2t_v, i, cols, (c, c + width)))
                    for t in range(c, c + width, 128):
                        part = n[:, t - c:t - c + 128]
                        acc[i, t] = acc[i, t] + part if (i, t) in acc else part
                    return jnp.concatenate([acc[i, t] for t in range(c, c + width, 128)], axis=1)

                def emit_out(i, j, v):
                    rows = half_rows(it, TC, i)
                    out_v[rows, j * D2 + c:j * D2 + c + width] = (
                        h_v[j][rows, c:c + width] + b2[:, j * D2 + c:j * D2 + c + width] + v).astype(BF)
                if last:
                    _strassen(prod, emit_out)
                else:
                    for i in (2, 4, 5, 1, 3, 0, 6):
                        prod(i)

        pending = []
        for cols in FCH:
            pending.append((cols, hidden(cols)))
            if len(pending) > CFG["c2_skew"]:
                project(*pending.pop(0), last=cols == FCH[-1] and not pending)
        while pending:
            item = pending.pop(0)
            project(*item, last=not pending)
        out_copy(it).start()
        return carry
    with _scope("C2"):
        _ln_stats(jnp.concatenate([h_v[0][0:TC, :], h_v[1][0:TC, :]], axis=1), stat_v)
        lax.fori_loop(0, S // TC, mlp_body, 0)
    with _scope("outwait"):
        for i in range(S // TC):
            out_copy(i).wait()


@jax.jit
def pallas_sequential_preLN__softmax_full_mha__mixer_channel_mlp__prompt_kernel(A_x, A_wqkv, A_wo, B_x, B_w1, B_b1, B_w2, B_b2):
    del B_x
    any_spec = pl.BlockSpec(memory_space=pl.ANY)
    out = pl.pallas_call(
        _kernel,
        out_shape=jax.ShapeDtypeStruct((S, D), BF),
        in_specs=[any_spec] * 7,
        out_specs=any_spec,
        scratch_shapes=[
            pltpu.VMEM((S, D), BF),
            pltpu.VMEM((4, D, D), BF),
            pltpu.VMEM((4, 5, D2 // 2, D2), I32),
            pltpu.VMEM((D, F), BF),
            pltpu.VMEM((5, D2 // 2, F2), I32),
            pltpu.VMEM((F,), BF),
            pltpu.VMEM((F, D), BF),
            pltpu.VMEM((5, F2 // 2, D2), I32),
            pltpu.VMEM((D + 1536,), BF),
            pltpu.VMEM((NB, 7, TM // 4, D2), I32),
            pltpu.VMEM((2, NB, G, 64, TM), I32),
            pltpu.VMEM((G, S // 2, 128), I32),
            pltpu.VMEM((S, TM), F32),
            pltpu.VMEM((S, TM), F32),
            pltpu.VMEM((96, TM), F32),
            pltpu.VMEM((8, TM), F32),
            pltpu.VMEM((G, S, 128), F32),
            pltpu.VMEM((2, TM, 128), F32),
            pltpu.VMEM((S, D), BF),
            pltpu.SemaphoreType.DMA((NB,)),
            pltpu.SemaphoreType.DMA((4,)),
            pltpu.SemaphoreType.DMA((D // 128,)),
            pltpu.SemaphoreType.DMA((4,)),
            pltpu.SemaphoreType.DMA((S // TC,)),
        ],
        compiler_params=pltpu.CompilerParams(vmem_limit_bytes=120 * 1024 * 1024),
        name="fused_block",
    )(A_x.reshape(S, D), A_wqkv, A_wo, B_w1, B_b1, B_w2, B_b2)
    return out.reshape(1, S, D)
```

```python
import functools
import math

import jax
import jax.numpy as jnp
from jax import lax
import jax.experimental.pallas as pl
import jax.experimental.pallas.tpu as pltpu

S, D, F, DH = 2048, 1024, 3584, 32
G = D // 128
TM = 512
NB = S // TM
TC = 256
CK = 128
NC = S // CK
D2, D4, F4 = D // 2, D // 4, F // 4
EPS = 1e-5
QSCALE = (DH ** -0.5) * math.log2(math.e)
BF, F32, I32 = jnp.bfloat16, jnp.float32, jnp.int32


def _rows(i, n):
    return pl.ds(pl.multiple_of(i * n, n), n)


def _half_rows(r, n, i):
    return pl.ds(pl.multiple_of(r * n + i * (n // 2), n // 2), n // 2)


def _dot(a, b):
    return jnp.dot(a, b, preferred_element_type=F32)


def _pack(x):
    return pltpu.bitcast(x, I32)


def _unpack(x):
    return pltpu.bitcast(x, BF)


def _ln_stats(x, stat_ref, r0=0):
    m = jnp.mean(x, axis=-1, keepdims=True)
    xc = x - m
    v = jnp.mean(xc * xc, axis=-1, keepdims=True)
    n = x.shape[0]
    stat_ref[0, r0:r0 + n, :] = jnp.broadcast_to(m, (n, 128))
    stat_ref[1, r0:r0 + n, :] = jnp.broadcast_to(lax.rsqrt(v + EPS), (n, 128))


def _ln_apply(x, stat_ref, r0):
    n, reps = x.shape[0], (1, x.shape[1] // 128)
    return (x - jnp.tile(stat_ref[0, r0:r0 + n, :], reps)) * jnp.tile(stat_ref[1, r0:r0 + n, :], reps)


def _gelu(x):
    c = math.sqrt(2.0 / math.pi)
    inner = x * (c + (c * 0.044715) * (x * x))
    hx = 0.5 * x
    return hx + hx * jnp.tanh(inner)


class _Order:
    def __init__(self, step):
        self.true = lax.broadcasted_iota(I32, (8, 128), 0) >= jnp.minimum(step, 0)

    def tie(self, x, dep):
        packed = x.dtype != F32
        v = pltpu.bitcast(x, F32) if packed else x
        reps = (v.shape[0] // 8, v.shape[1] // 128)
        v = jnp.where(jnp.tile(self.true, reps), v, jnp.tile(dep, reps))
        return pltpu.bitcast(v, x.dtype) if packed else v

    def tie_first(self, x, dep):
        first = jnp.concatenate([self.tie(x[:16, :128], dep), x[:16, 128:]], axis=1)
        return jnp.concatenate([first, x[16:]], axis=0)

    def join(self, values):
        dep = None
        for x in values:
            v = pltpu.bitcast(x, F32) if x.dtype != F32 else x
            for i in range(0, v.shape[0], 8):
                for j in range(0, v.shape[1], 128):
                    t = v[i:i + 8, j:j + 128]
                    dep = t if dep is None else jnp.where(self.true, dep, t)
        return dep


class _Steps:
    def __init__(self, order, side, lag=0):
        self.order, self.side, self.lag, self.done = order, side, lag, []

    def __call__(self, a, b):
        if self.lag and len(self.done) >= self.lag and self.done[-self.lag]:
            a = self.order.tie_first(a, self.order.join(self.done[-self.lag]))
        d = _dot(a, b)
        job = self.side.get(len(self.done))
        self.done.append(job(d[0:8, 0:128]) if job else None)
        return d


class _Quad(tuple):
    def __add__(self, other):
        return _Quad(a + b for a, b in zip(self, other))

    def __sub__(self, other):
        return _Quad(a - b for a, b in zip(self, other))


def _left(a11, a12, a21, a22):
    return a11 + a22, a21 + a22, a11, a22, a11 + a12, a21 - a11, a12 - a22


def _right(b11, b12, b21, b22):
    return b11 + b22, b11, b12 - b22, b21 - b11, b22, b11 + b12, b21 + b22


_PRODUCT_ORDER = (2, 4, 1, 3, 0, 6, 5)


def _strassen(prod, emit):
    m3, m5 = prod(2), prod(4)
    emit(0, 1, m3 + m5)
    m2, m4 = prod(1), prod(3)
    emit(1, 0, m2 + m4)
    t22, t11 = m3 - m2, m4 - m5
    m1, m7 = prod(0), prod(6)
    emit(0, 0, t11 + m1 + m7)
    emit(1, 1, t22 + m1 + prod(5))


def _weight_terms(w_ref, t_ref, i, n, order, dep):
    top, bottom = _rows(i, n), pl.ds(pl.multiple_of(D2 + i * n, n), n)
    right = _right(*[order.tie(w_ref[rows, c:c + D2], dep).astype(F32)
                     for rows in (top, bottom) for c in (0, D2)])
    terms = [right[k].astype(BF) for k in (0, 2, 3, 5, 6)]
    for s, t in enumerate(terms):
        t_ref[s, _rows(i, n // 2), :] = _pack(t)
    return terms


def _project(step, lhs, w_ref, t_ref, emit):
    def rhs(i, c):
        if i == 1:
            return w_ref[0:D2, c:c + 128]
        if i == 4:
            return w_ref[D2:D, D2 + c:D2 + c + 128]
        return _unpack(t_ref[{0: 0, 2: 1, 3: 2, 5: 3, 6: 4}[i], :, c:c + 128])
    for c in range(0, D2, 128):
        _strassen(lambda i: step(lhs(i), rhs(i, c)), functools.partial(emit, c // 128))


def _left_terms2(block):
    quads = [_Quad(block(2 * a + i, 2 * b + j) for i in range(2) for j in range(2))
             for a in range(2) for b in range(2)]
    return [t.astype(BF) for outer in _left(*quads) for t in _left(*outer)]


def _weight_terms2(w_ref, t_ref, i, c0, order, dep):
    k4, n4 = w_ref.shape[0] // 4, w_ref.shape[1] // 4

    def quad(a, b, dep):
        def block(a, b):
            rows = pl.ds(pl.multiple_of(a * k4 + i * 16, 16), 16)
            return order.tie(w_ref[rows, b * n4 + c0:b * n4 + c0 + 128], dep).astype(F32)
        return _Quad(block(2 * a + k // 2, 2 * b + k % 2) for k in range(4))

    def store(p, outer):
        for q, t in enumerate(_right(*outer)):
            t = _pack(t.astype(BF))
            t_ref[7 * p + q, _rows(i, 8), c0:c0 + 128] = t
        return pltpu.bitcast(t, F32)

    b11 = quad(0, 0, dep)
    dep = store(1, b11)
    b22 = quad(1, 1, dep)
    store(0, b11 + b22)
    dep = store(4, b22)
    b12 = quad(0, 1, dep)
    store(2, b12 - b22)
    dep = store(5, b11 + b12)
    b21 = quad(1, 0, dep)
    store(3, b21 - b11)
    return [store(6, b21 + b22)]


def _strassen2(prod, emit):
    def outer(p):
        res = {}
        _strassen(lambda q: prod(7 * p + q), lambda i, j, v: res.update({(i, j): v}))
        return _Quad(res[i, j] for i in range(2) for j in range(2))

    def emit_quad(a, b, quad):
        for k, v in enumerate(quad):
            emit(2 * a + k // 2, 2 * b + k % 2, v)
    _strassen(outer, emit_quad)


def _kernel(x_hbm, wqkv_hbm, wo_hbm, w1_hbm, b1_hbm, w2_hbm, b2_hbm, out_hbm,
            x_v, w_v, wt_v, w1_v, w1t_v, b1_v, w2_v, w2t_v, b2_v,
            y_v, qvt_v, k_v, sa_v, sb_v, ot_v, l_v, o_v, stat_v, tail_v,
            sem_x, sem_w, sem_k, sem_m, sem_o):
    WQ, WK, WV, WO = range(4)

    def x_copy(r):
        return pltpu.make_async_copy(x_hbm.at[_rows(r, TM), :], x_v.at[_rows(r, TM), :], sem_x.at[r])

    def wk_copy(i, half):
        rows = pl.ds(pl.multiple_of(half * D2 + i * 128, 128), 128)
        return pltpu.make_async_copy(wqkv_hbm.at[rows, pl.ds(WK * D, D)], w_v.at[WK, rows, :],
                                     sem_k.at[2 * i + half])

    w_copy = {c: pltpu.make_async_copy(wqkv_hbm.at[:, pl.ds(c * D, D)], w_v.at[c], sem_w.at[c])
              for c in (WQ, WV)}
    w_copy[WO] = pltpu.make_async_copy(wo_hbm, w_v.at[WO], sem_w.at[WO])
    w1_copy, *late_copies = [
        pltpu.make_async_copy(src, dst, sem_m.at[i]) for i, (src, dst) in enumerate(
            [(w1_hbm, w1_v), (w2_hbm, w2_v), (b1_hbm, b1_v), (b2_hbm, b2_v.at[pl.ds(0, D)])])]

    def prepare_weight(c, wait=None):
        def body(i, carry):
            if wait:
                pl.when(i % 4 == 0)(lambda: wait(i // 4))
            _weight_terms(w_v.at[c], wt_v.at[c], i, 32, _Order(i), jnp.zeros((8, 128), F32))
            return carry
        lax.fori_loop(0, D2 // 32, body, 0)

    def wk_start(i):
        wk_copy(i, 0).start()
        wk_copy(i, 1).start()

    def wk_wait(i):
        wk_copy(i, 0).wait()
        wk_copy(i, 1).wait()
        pl.when(i + 2 < D2 // 128)(lambda: wk_start(i + 2))
        pl.when(i + 2 == D2 // 128)(lambda: x_copy(1).start())

    x_copy(0).start()
    wk_start(0)
    sa_v[:, 256:] = jnp.zeros((S, 256), F32)
    sb_v[:, 256:] = jnp.zeros((S, 256), F32)
    ot_v[...] = jnp.zeros_like(ot_v)
    l_v[...] = jnp.ones_like(l_v)
    tail_v[...] = jnp.zeros_like(tail_v)
    x_copy(0).wait()
    wk_start(1)
    _ln_stats(x_v[0:TM, :].astype(F32), stat_v)
    prepare_weight(WK, wk_wait)
    x_copy(2).start()
    x_copy(3).start()
    w_copy[WQ].start()
    w_copy[WV].start()

    def k_body(r, carry):
        nxt = jnp.minimum(r + 1, NB - 1)
        pl.when(r + 1 < NB)(lambda: x_copy(nxt).wait())

        @pl.when(r == 1)
        def _():
            w_copy[WO].start()
            w1_copy.start()

        order = _Order(r)
        y = [_ln_apply(x_v[_half_rows(r, TM, i), c:c + D2].astype(F32), stat_v, i * (TM // 2))
             for i in range(2) for c in (0, D2)]
        for i, t in enumerate(_left(*y)):
            y_v[r, i] = _pack(t.astype(BF))

        def next_stats(k, dep):
            _ln_stats(order.tie(x_v[_rows(16 * nxt + k, 32), :], dep).astype(F32), stat_v, 32 * k)

        def emit(n, i, j, v):
            k_v[4 * j + n, _half_rows(r, TM // 2, i), :] = _pack(v.astype(BF))
        side = {10 + k: functools.partial(next_stats, k) for k in range(16)}
        _project(_Steps(order, side), lambda i: _unpack(y_v[r, i]), w_v.at[WK], wt_v.at[WK], emit)
        return carry
    lax.fori_loop(0, NB, k_body, 0)

    w_copy[WQ].wait()
    prepare_weight(WQ)
    w_copy[WV].wait()
    w_copy[WO].wait()
    w1_copy.wait()
    for cp in late_copies:
        cp.start()

    def qv_write(it, n, i, j, v):
        which, r = it // NB, it % NB
        scale = jnp.where(which == 0, QSCALE, 1.0).astype(F32)
        qvt_v[which, r, 4 * j + n, :, i * (TM // 2):(i + 1) * (TM // 2)] = _pack((v * scale).T.astype(BF))

    def qv_flush(it):
        for i in range(2):
            qv_write(it, G // 2 - 1, i, i, tail_v[i])

    def qv_body(it, carry):
        which, r = it // NB, it % NB
        qv_flush(jnp.maximum(it - 1, 0))

        def emit(n, i, j, v):
            if n == G // 2 - 1 and i == j:
                tail_v[i] = v
            else:
                qv_write(it, n, i, j, v)
        order = _Order(it)
        side = [functools.partial(_weight_terms, w_v.at[WV + which], wt_v.at[WV + which], 8 * r + i, 16, order)
                for i in range(8)]
        side += [functools.partial(_weight_terms2, w1_v, w1t_v, 2 * it + i, c, order)
                 for i in range(2) for c in range(0, F4, 128)]
        _project(_Steps(order, dict(enumerate(side)), 2), lambda i: _unpack(y_v[r, i]),
                 w_v.at[2 * which], wt_v.at[2 * which], emit)
        return carry
    lax.fori_loop(0, 2 * NB, qv_body, 0)
    qv_flush(2 * NB - 1)

    scores = (sa_v, sb_v)

    def q_weights(t, j):
        parts = [_unpack(qvt_v[0, t // G, t % G, 16 * j:16 * (j + 1), :])]
        if j > 0:
            parts.insert(0, jnp.zeros((DH * j, TM), BF))
        if j < 3:
            parts.append(jnp.zeros((DH * (3 - j), TM), BF))
        return jnp.concatenate(parts, axis=0)

    def score_chunk(t, j, c, qw, mp):
        s = _dot(_unpack(k_v[t % G, c * CK // 2:(c + 1) * CK // 2, :]), qw)
        for half, ref in enumerate(scores):
            ref[c * CK:(c + 1) * CK, (j % 2) * 256:(j % 2 + 1) * 256] = s[:, half * 256:(half + 1) * 256]
        for i in range(0, CK, 8):
            mp = s[i:i + 8] if mp is None else jnp.maximum(mp, s[i:i + 8])
        return mp

    def softmax_chunk(t, j, c, m, l, pace=None):
        ps = []
        for k in range(2):
            s = jnp.concatenate([ref[c * CK + k * 64:c * CK + (k + 1) * 64, (j % 2) * 256:(j % 2 + 1) * 256]
                                 for ref in scores], axis=1)
            p = jnp.exp2(s.reshape(8, 8, TM) - (pace(k, m, l) if pace else m)[None])
            terms = [p[i] for i in range(8)]
            while len(terms) > 1:
                terms = [a + b for a, b in zip(terms[0::2], terms[1::2])]
            l = terms[0] if l is None else l + terms[0]
            ps.append(p.reshape(64, TM))
        block, col = divmod(c * CK, TM)
        vt = _unpack(qvt_v[1, block, t % G, 16 * j:16 * (j + 1), col:col + CK])
        return _dot(vt, jnp.concatenate(ps, axis=0).astype(BF)), l

    def normalise(acc, l):
        return acc * (1.0 / jnp.sum(l, axis=0, keepdims=True))

    def finish_group(t, acc, l):
        ot = jnp.concatenate([ot_v[0:64, :], normalise(ot_v[64:96, :], l_v[...]), normalise(acc, l)], axis=0)
        o = ot.T
        o_v[t % G, _rows(t // G, TM), :] = o
        return jnp.concatenate([o[i + 120:i + 128, :] for i in range(0, TM, 128)], axis=1)

    def attention_body(t, carry):
        m, mp = carry
        prev, nxt = jnp.maximum(t - 1, 0), jnp.minimum(t + 1, NB * G - 1)
        sublane = lax.broadcasted_iota(I32, (8, TM), 0)
        true1, true2 = sublane >= jnp.minimum(t, 0), sublane < 8 + jnp.maximum(t, 0)
        qw = q_weights(t, 0)
        m_next = finished = None
        sums, outs = [], []
        for step, (tc, j) in enumerate(((prev, 3), (t, 0), (t, 1), (t, 2))):
            l = acc = None
            m = jnp.broadcast_to(m, (8, TM))
            for c in range(NC):
                u = step * NC + c
                js, cs = divmod(u + 1, NC)
                ts, js = (t, js) if js < 4 else (nxt, 0)
                if cs == 0:
                    qw, mp = q_weights(ts, js), None
                mp = score_chunk(ts, js, cs, qw, mp)
                if cs == NC - 1:
                    m_next = jnp.max(mp, axis=0, keepdims=True)

                def pace(k, m, l):
                    if l is not None:
                        sums.append(l)
                    if len(sums) >= 3:
                        m = jnp.where(true1, m, sums[-3])
                    if k == 0 and u >= 2:
                        m = jnp.where(true2, m, outs[u - 2][0:8, :])
                    if k == 1 and u == NC + 3:
                        m = jnp.where(true2, m, finished)
                    return m
                o, l = softmax_chunk(tc, j, c, m, l, pace)
                outs.append(o)
                acc = o if acc is None else acc + o
            sums.append(l)
            if j == 3:
                finished = finish_group(tc, acc, l)
            elif j < 2:
                ot_v[DH * j:DH * (j + 1), :] = normalise(acc, l)
            else:
                ot_v[64:96, :] = acc
                l_v[...] = l
            m = m_next
        return m, mp

    for cp in late_copies:
        cp.wait()
    mp = score_chunk(0, 0, 0, q_weights(0, 0), None)
    m, _ = lax.fori_loop(0, NB * G, attention_body, (jnp.zeros((1, TM), F32), mp))
    l = acc = None
    for c in range(NC):
        o, l = softmax_chunk(NB * G - 1, 3, c, jnp.broadcast_to(m, (8, TM)), l)
        acc = o if acc is None else acc + o
    finish_group(NB * G - 1, acc, l)

    h_v = scores

    def wo_body(r, carry):
        o = [jnp.concatenate([o_v[4 * j + g, _half_rows(r, TM, i), :] for g in range(G // 2)], axis=1)
             for i in range(2) for j in range(2)]
        lhs = [t.astype(BF) for t in _left(*o)]

        def emit(n, i, j, v):
            rows, c = _half_rows(r, TM, i), n * 128
            h_v[j][rows, c:c + 128] = x_v[rows, j * D2 + c:j * D2 + c + 128].astype(F32) + v
        order = _Order(r)

        def w2_terms(k, dep):
            first = _weight_terms2(w2_v, w2t_v, 14 * r + k, 0, order, dep)
            return first + _weight_terms2(w2_v, w2t_v, 14 * r + k, 128, order, first[0])
        side = {9 + k: functools.partial(w2_terms, k) for k in range(14)}
        _project(_Steps(order, side, 2), lambda i: lhs[i], w_v.at[WO], wt_v.at[WO], emit)
        return carry
    lax.fori_loop(0, NB, wo_body, 0)

    out_v = x_v

    def out_copy(i):
        return pltpu.make_async_copy(out_v.at[_rows(i, TC), :], out_hbm.at[_rows(i, TC), :], sem_o.at[i])

    def mlp_body(it, carry):
        b1 = b1_v[...].astype(F32).reshape(1, F)
        b2 = b2_v[pl.ds(0, D)].astype(F32).reshape(1, D)
        n = TC // 4

        def rows(a):
            return pl.ds(pl.multiple_of(it * TC + a * n, n), n)

        def h_block(a, b):
            return h_v[b // 2][rows(a), (b % 2) * D4:(b % 2 + 1) * D4]
        y = _left_terms2(lambda a, b: _ln_apply(h_block(a, b), stat_v, a * n))
        order = _Order(it)

        def next_stats(k, dep):
            part = _rows(8 * jnp.minimum(it + 1, S // TC - 1) + k, 32)
            _ln_stats(order.tie(jnp.concatenate([h_v[0][part, :], h_v[1][part, :]], axis=1), dep), stat_v, 32 * k)
        step = _Steps(order, {60 + 8 * k: functools.partial(next_stats, k) for k in range(8)})

        hidden = []
        for c in range(0, F4, 128):
            g = {}

            def emit_hidden(a, b, v):
                g[a, b] = _gelu(v + b1[:, b * F4 + c:b * F4 + c + 128])
            _strassen2(lambda s: step(y[s], _unpack(w1t_v[s, :, c:c + 128])), emit_hidden)
            hidden.append(_left_terms2(lambda a, b: g[a, b]))

        def down(s, t0, t1):
            lhs = jnp.concatenate([tile[s] for tile in hidden[t0:t1]], axis=1)
            return step(lhs, _unpack(w2t_v[s, t0 * 64:t1 * 64, :]))
        first = {7 * p + q: down(7 * p + q, 0, 3) for p in _PRODUCT_ORDER for q in _PRODUCT_ORDER}

        def emit_out(a, b, v):
            out_v[rows(a), b * D4:(b + 1) * D4] = (h_block(a, b) + b2[:, b * D4:(b + 1) * D4] + v).astype(BF)
        _strassen2(lambda s: first[s] + down(s, 3, F4 // 128), emit_out)
        out_copy(it).start()
        return carry

    _ln_stats(jnp.concatenate([h_v[0][0:TC, :], h_v[1][0:TC, :]], axis=1), stat_v)
    lax.fori_loop(0, S // TC, mlp_body, 0)
    for i in range(S // TC):
        out_copy(i).wait()


@jax.jit
def pallas_sequential_preLN__softmax_full_mha__mixer_channel_mlp__prompt_kernel(
    A_x: jax.Array,
    A_wqkv: jax.Array,
    A_wo: jax.Array,
    B_x: jax.Array,
    B_w1: jax.Array,
    B_b1: jax.Array,
    B_w2: jax.Array,
    B_b2: jax.Array,
):
    del B_x
    any_spec = pl.BlockSpec(memory_space=pl.ANY)
    out = pl.pallas_call(
        _kernel,
        out_shape=jax.ShapeDtypeStruct((S, D), BF),
        in_specs=[any_spec] * 7,
        out_specs=any_spec,
        scratch_shapes=[
            pltpu.VMEM((S, D), BF),
            pltpu.VMEM((4, D, D), BF),
            pltpu.VMEM((4, 5, D2 // 2, D2), I32),
            pltpu.VMEM((D, F), BF),
            pltpu.VMEM((49, D4 // 2, F4), I32),
            pltpu.VMEM((F,), BF),
            pltpu.VMEM((F, D), BF),
            pltpu.VMEM((49, F4 // 2, D4), I32),
            pltpu.VMEM((D + 1536,), BF),
            pltpu.VMEM((NB, 7, TM // 4, D2), I32),
            pltpu.VMEM((2, NB, G, 64, TM), I32),
            pltpu.VMEM((G, S // 2, 128), I32),
            pltpu.VMEM((S, TM), F32),
            pltpu.VMEM((S, TM), F32),
            pltpu.VMEM((3 * DH, TM), F32),
            pltpu.VMEM((8, TM), F32),
            pltpu.VMEM((G, S, 128), F32),
            pltpu.VMEM((2, TM, 128), F32),
            pltpu.VMEM((2, TM // 2, 128), F32),
            pltpu.SemaphoreType.DMA((NB,)),
            pltpu.SemaphoreType.DMA((4,)),
            pltpu.SemaphoreType.DMA((D // 128,)),
            pltpu.SemaphoreType.DMA((4,)),
            pltpu.SemaphoreType.DMA((S // TC,)),
        ],
        compiler_params=pltpu.CompilerParams(vmem_limit_bytes=126 * 1024 * 1024),
        name="fused_block",
    )(A_x.reshape(S, D), A_wqkv, A_wo, B_w1, B_b1, B_w2, B_b2)
    return out.reshape(1, S, D)
```
